```python
import os as _os
_os.environ.setdefault("JAX_PLATFORMS", "cpu")
import jax
import jax.numpy as jnp

def _softmax(x, axis=-1):
    return jax.nn.softmax(x, axis=axis)
def _gelu(x):
    return jax.nn.gelu(x, approximate=True)
def _silu(x):
    return jax.nn.silu(x)
def _sigmoid(x):
    return jax.nn.sigmoid(x)
def _layernorm(x, axis=-1, eps=1e-5):
    m = jnp.mean(x, axis=axis, keepdims=True)
    v = jnp.var(x, axis=axis, keepdims=True)
    return (x - m) / jnp.sqrt(v + eps)
def _scatter_add(tgt, idx, src, axis=0):
    return tgt.at[idx].add(src)
def _segment_sum(src, seg, n):
    return jax.ops.segment_sum(src, seg, n)
class _Rng:
    def __init__(self, key):
        self._k = key
    def _next(self):
        self._k, sub = jax.random.split(self._k)
        return sub
    def normal(self, shape):
        return jax.random.normal(self._next(), shape, dtype=jnp.bfloat16)
    def randint(self, lo, hi, shape):
        return jax.random.randint(self._next(), shape, lo, hi, dtype=jnp.int32)
    def uniform(self, shape, lo=0.0, hi=1.0):
        return jax.random.uniform(self._next(), shape, jnp.bfloat16, lo, hi)
    def permutation(self, n):
        return jax.random.permutation(self._next(), n)


kernel_name = 'gated_mix__grouped_kv_mqa__ssm_conv_s5__prompt'

def setup_inputs():
    _rng = _Rng(jax.random.key(int.from_bytes(__import__("os").urandom(4), "little")))
    _w = (lambda a: (lambda t: t.astype(jnp.bfloat16) if jnp.issubdtype(t.dtype, jnp.floating) else t)(jnp.asarray(a)))
    def _A_setup():
        B, S, D, H = 1, 2048, 512, 32
        Dh = D // H
        return {
            "x": _w((lambda *s: _rng.normal(s) * 0.05)(B, S, D)),
            "wq": _w((lambda *s: _rng.normal(s) * 1.6)(D, H * Dh)),
            "wk": _w((lambda *s: _rng.normal(s) * 1.6)(D, Dh)),
            "wv": _w((lambda *s: _rng.normal(s) * 0.05)(D, Dh)),
            "wo": _w((lambda *s: _rng.normal(s) * 0.05)(H * Dh, D)),
        }
    _A_in = _A_setup()

    def _B_setup():
        B, S, D = 1, 2048, 512
        P = D
        Lambda_re = -0.5 * jnp.exp((lambda *s: _rng.normal(s) * 0.4)(P))
        Lambda_im = (lambda *s: _rng.normal(s) * 0.4)(P) * 1.0
        B_re = (lambda *s: _rng.normal(s) * 0.4)(P, D) * (D ** -0.5)
        B_im = (lambda *s: _rng.normal(s) * 0.4)(P, D) * (D ** -0.5)
        C_re = (lambda *s: _rng.normal(s) * 0.4)(D, P) * (P ** -0.5)
        C_im = (lambda *s: _rng.normal(s) * 0.4)(D, P) * (P ** -0.5)
        log_dt = (lambda *s: _rng.normal(s) * 0.4)(P) * 0.3 - 2.0
        Dskip = (lambda *s: _rng.normal(s) * 0.4)(D)
        return {
            "x": _w((lambda *s: _rng.normal(s) * 0.05)(B, S, D)),
            "Lambda_re": _w(Lambda_re),
            "Lambda_im": _w(Lambda_im),
            "B_re": _w(B_re),
            "B_im": _w(B_im),
            "C_re": _w(C_re),
            "C_im": _w(C_im),
            "log_dt": _w(log_dt),
            "Dskip": _w(Dskip),
        }
    _B_in = _B_setup()

    return {
        "A_x": _A_in["x"],
        "A_wq": _A_in["wq"],
        "A_wk": _A_in["wk"],
        "A_wv": _A_in["wv"],
        "A_wo": _A_in["wo"],
        "B_x": _B_in["x"],
        "B_Lambda_re": _B_in["Lambda_re"],
        "B_Lambda_im": _B_in["Lambda_im"],
        "B_B_re": _B_in["B_re"],
        "B_B_im": _B_in["B_im"],
        "B_C_re": _B_in["C_re"],
        "B_C_im": _B_in["C_im"],
        "B_log_dt": _B_in["log_dt"],
        "B_Dskip": _B_in["Dskip"],
        "gate_w": _w((lambda *s: _rng.normal(s) * 0.05)(512) * 16.0),
    }

def reference(A_x, A_wq, A_wk, A_wv, A_wo, B_x, B_Lambda_re, B_Lambda_im, B_B_re, B_B_im, B_C_re, B_C_im, B_log_dt, B_Dskip, gate_w):
    def _A_ref(x, wq, wk, wv, wo):
        B, S, D = x.shape
        H = 32
        Dh = D // H
        q = (lambda x, *d: x.transpose(*d))((x @ wq).reshape(B, S, H, Dh), 0, 2, 1, 3)
        k = x @ wk
        v = x @ wv
        scores = jnp.einsum("bhqd,bkd->bhqk", q, k) * (Dh ** -0.5)
        p = _softmax(scores, axis=-1)
        o = jnp.einsum("bhqk,bkd->bhqd", p, v)
        return (lambda x, *d: x.transpose(*d))(o, 0, 2, 1, 3).reshape(B, S, H * Dh) @ wo

    def _B_ref(x, Lambda_re, Lambda_im, B_re, B_im, C_re, C_im, log_dt, Dskip):
        Bsz, L, H = x.shape
        Lam = Lambda_re + 1j * Lambda_im
        Bmat = B_re + 1j * B_im
        Cmat = C_re + 1j * C_im
        dt = jnp.exp(log_dt)
        Lam_bar = jnp.exp(dt * Lam)
        B_bar = ((Lam_bar - 1.0) / Lam)[:, None] * Bmat
        Bu = jnp.einsum("bld,pd->blp", x + 0j, B_bar)
        h = jnp.zeros_like(Bu[:, 0, :])
        hs = []
        for t in range(L):
            h = Lam_bar[None, :] * h + Bu[:, t, :]
            hs.append(h)
        hseq = jnp.stack(hs, 1)
        y = 2.0 * jnp.einsum("blp,dp->bld", hseq, Cmat).real + x * Dskip[None, None, :]
        return y

    x = A_x
    g = _sigmoid((x * gate_w).sum(-1, keepdims=True))
    a = _A_ref(x, A_wq, A_wk, A_wv, A_wo)
    b = _B_ref(x, B_Lambda_re, B_Lambda_im, B_B_re, B_B_im, B_C_re, B_C_im, B_log_dt, B_Dskip)
    return g * a + (1 - g) * b
```

```python
import jax
import jax.numpy as jnp
import jax.experimental.pallas as pl
import jax.experimental.pallas.tpu as pltpu

S = 2048
D = 512
H = 32
DH = 16
P = 512
NQ = 512
CK = 128
NSEG = 8
SEGLEN = S // NSEG
NG = P // 128

_NT = (((1,), (1,)), ((), ()))


def _bf(v):
    return v.astype(jnp.bfloat16)


def _kernel(x_ref, wq_ref, wk_ref, wv_ref, wo_ref, lre_ref, lim_ref, ldt_ref,
            bre_ref, bim_ref, cre_ref, cim_ref, dsk_ref, gw_ref,
            o_ref,
            qt_s, k_s, vt_s, y_s, ure_s, uim_s, ot_s, sA, sB):
    i = pl.program_id(0)

    @pl.when(i == 0)
    def _prologue():
        x = x_ref[...]
        q = jnp.dot(x, wq_ref[...], preferred_element_type=jnp.float32) * (DH ** -0.5)
        qt_s[...] = _bf(q.T)
        k_s[...] = _bf(jnp.dot(x, wk_ref[...], preferred_element_type=jnp.float32))
        v = jnp.dot(x, wv_ref[...], preferred_element_type=jnp.float32)
        vt_s[...] = _bf(v.T)

        lr = lre_ref[...].astype(jnp.float32)
        li = lim_ref[...].astype(jnp.float32)
        dt = _bf(jnp.exp(ldt_ref[...].astype(jnp.float32))).astype(jnp.float32)
        mag = jnp.exp(dt * lr)
        ang = dt * li
        lb_re = mag * jnp.cos(ang)
        lb_im = mag * jnp.sin(ang)
        nr = lb_re - 1.0
        ni = lb_im
        den = lr * lr + li * li
        cf_re = (nr * lr + ni * li) / den
        cf_im = (ni * lr - nr * li) / den

        u_re = jax.lax.dot_general(x, bre_ref[...], _NT, preferred_element_type=jnp.float32)
        u_im = jax.lax.dot_general(x, bim_ref[...], _NT, preferred_element_type=jnp.float32)
        bu_re = cf_re * u_re - cf_im * u_im
        bu_im = cf_re * u_im + cf_im * u_re
        for g in range(NG):
            ure_s[g] = bu_re[:, 128 * g:128 * (g + 1)]
            uim_s[g] = bu_im[:, 128 * g:128 * (g + 1)]

        def grp(a, g):
            return a[:, 128 * g:128 * (g + 1)]

        lbr = [jnp.broadcast_to(grp(lb_re, g), (NSEG, 128)) for g in range(NG)]
        lbi = [jnp.broadcast_to(grp(lb_im, g), (NSEG, 128)) for g in range(NG)]

        def seg_rows(j):
            return pl.ds(j, NSEG, stride=SEGLEN)

        def local_step(j, c):
            out = []
            for g in range(NG):
                hr, hi = c[g]
                br = ure_s[g, seg_rows(j), :]
                bi = uim_s[g, seg_rows(j), :]
                out.append((lbr[g] * hr - lbi[g] * hi + br, lbr[g] * hi + lbi[g] * hr + bi))
            return tuple(out)

        z = jnp.zeros((NSEG, 128), jnp.float32)
        ends = jax.lax.fori_loop(0, SEGLEN, local_step, tuple((z, z) for _ in range(NG)), unroll=8)

        pr, pi_ = lb_re, lb_im
        for _ in range(8):
            pr, pi_ = pr * pr - pi_ * pi_, 2.0 * pr * pi_
        inits = []
        for g in range(NG):
            er, ei = ends[g]
            prg, pig = grp(pr, g), grp(pi_, g)
            cr = jnp.zeros((1, 128), jnp.float32)
            ci = jnp.zeros((1, 128), jnp.float32)
            rr, ri = [cr], [ci]
            for sgi in range(1, NSEG):
                e_r = er[sgi - 1:sgi, :]
                e_i = ei[sgi - 1:sgi, :]
                cr, ci = prg * cr - pig * ci + e_r, prg * ci + pig * cr + e_i
                rr.append(cr)
                ri.append(ci)
            inits.append((jnp.concatenate(rr, axis=0), jnp.concatenate(ri, axis=0)))

        def true_step(j, c):
            out = []
            for g in range(NG):
                hr, hi = c[g]
                nhr = lbr[g] * hr - lbi[g] * hi + ure_s[g, seg_rows(j), :]
                nhi = lbr[g] * hi + lbi[g] * hr + uim_s[g, seg_rows(j), :]
                ure_s[g, seg_rows(j), :] = nhr
                uim_s[g, seg_rows(j), :] = nhi
                out.append((nhr, nhi))
            return tuple(out)

        jax.lax.fori_loop(0, SEGLEN, true_step, tuple(inits), unroll=8)
        h_re = jnp.concatenate([ure_s[g] for g in range(NG)], axis=1)
        h_im = jnp.concatenate([uim_s[g] for g in range(NG)], axis=1)

        yy = (jax.lax.dot_general(_bf(h_re), cre_ref[...], _NT, preferred_element_type=jnp.float32)
              - jax.lax.dot_general(_bf(h_im), cim_ref[...], _NT, preferred_element_type=jnp.float32))
        skip = _bf(x.astype(jnp.float32) * dsk_ref[...].astype(jnp.float32)).astype(jnp.float32)
        y_s[...] = 2.0 * yy + skip

    q0 = pl.multiple_of(i * NQ, NQ)
    nck = S // CK

    def stage(h_qk, s_dst, h_sm, s_src, m):
        if h_qk is not None:
            qtn = qt_s[pl.ds(pl.multiple_of(h_qk * DH, DH), DH), pl.ds(q0, NQ)]
        if h_sm is not None:
            lrun = jnp.zeros((8, NQ), jnp.float32)
            acc = jnp.zeros((DH, NQ), jnp.float32)
        mrun = None
        for c in range(nck):
            if h_qk is not None:
                kc = k_s[pl.ds(c * CK, CK), :]
                sn = jnp.dot(kc, qtn, preferred_element_type=jnp.float32)
                s_dst[pl.ds(c * CK, CK), :] = sn
                cm = jnp.max(sn.reshape(CK // 8, 8, NQ), axis=0)
                mrun = cm if mrun is None else jnp.maximum(mrun, cm)
            if h_sm is not None:
                s = s_src[pl.ds(c * CK, CK), :]
                p = jnp.exp(s - m)
                lrun = lrun + jnp.sum(p.reshape(CK // 8, 8, NQ), axis=0)
                vc = vt_s[:, pl.ds(c * CK, CK)]
                acc = acc + jnp.dot(vc, _bf(p), preferred_element_type=jnp.float32)
        if h_sm is not None:
            l = jnp.sum(lrun, axis=0, keepdims=True)
            ot_s[pl.ds(pl.multiple_of(h_sm * DH, DH), DH), :] = acc / l
        if h_qk is not None:
            return jnp.max(mrun, axis=0, keepdims=True)
        return None

    m0 = stage(0, sA, None, None, None)

    def body(h, m):
        return jax.lax.cond(h % 2 == 0,
                            lambda mm: stage(h + 1, sB, h, sA, mm),
                            lambda mm: stage(h + 1, sA, h, sB, mm), m)

    m_last = jax.lax.fori_loop(0, H - 1, body, m0)
    stage(None, None, H - 1, sB, m_last)

    o_blk = _bf(ot_s[...].T)
    a = jnp.dot(o_blk, wo_ref[...], preferred_element_type=jnp.float32)
    xb = x_ref[pl.ds(q0, NQ), :].astype(jnp.float32)
    logit = jnp.sum(xb * gw_ref[...].astype(jnp.float32), axis=-1, keepdims=True)
    g = jax.nn.sigmoid(logit)
    o_ref[...] = g * a + (1.0 - g) * y_s[pl.ds(q0, NQ), :]


@jax.jit
def pallas_gated_mix__grouped_kv_mqa__ssm_conv_s5__prompt_kernel(
    A_x, A_wq, A_wk, A_wv, A_wo, B_x, B_Lambda_re, B_Lambda_im, B_B_re, B_B_im,
    B_C_re, B_C_im, B_log_dt, B_Dskip, gate_w,
):
    x = A_x.reshape(S, D)
    row = lambda a: a.reshape(1, -1)

    def full(shape):
        return pl.BlockSpec(shape, lambda i: (0,) * len(shape))

    out = pl.pallas_call(
        _kernel,
        grid=(S // NQ,),
        in_specs=[full((S, D)), full((D, H * DH)), full((D, DH)), full((D, DH)),
                  full((H * DH, D)), full((1, P)), full((1, P)), full((1, P)),
                  full((P, D)), full((P, D)), full((D, P)), full((D, P)),
                  full((1, D)), full((1, D))],
        out_specs=pl.BlockSpec((NQ, D), lambda i: (i, 0)),
        out_shape=jax.ShapeDtypeStruct((S, D), jnp.float32),
        scratch_shapes=[
            pltpu.VMEM((H * DH, S), jnp.bfloat16),
            pltpu.VMEM((S, DH), jnp.bfloat16),
            pltpu.VMEM((DH, S), jnp.bfloat16),
            pltpu.VMEM((S, D), jnp.float32),
            pltpu.VMEM((NG, S, 128), jnp.float32),
            pltpu.VMEM((NG, S, 128), jnp.float32),
            pltpu.VMEM((H * DH, NQ), jnp.float32),
            pltpu.VMEM((S, NQ), jnp.float32),
            pltpu.VMEM((S, NQ), jnp.float32),
        ],
        compiler_params=pltpu.CompilerParams(
            dimension_semantics=("arbitrary",),
            vmem_limit_bytes=100 * 1024 * 1024),
    )(x, A_wq, A_wk, A_wv, A_wo, row(B_Lambda_re), row(B_Lambda_im), row(B_log_dt),
      B_B_re, B_B_im, B_C_re, B_C_im, row(B_Dskip), row(gate_w))
    return out.reshape(1, S, D)
```

```python
import jax
import jax.numpy as jnp
import jax.experimental.pallas as pl
import jax.experimental.pallas.tpu as pltpu

S = 2048
D = 512
H = 32
DH = 16
P = 512
NQ = 512
CK = 128
LA = 2
NSEG = 8
SEGLEN = S // NSEG

_NT = (((1,), (1,)), ((), ()))


def _bf(v):
    return v.astype(jnp.bfloat16)


def _kernel(x_ref, wq_ref, wk_ref, wv_ref, wo_ref, lre_ref, lim_ref, ldt_ref,
            bre_ref, bim_ref, cre_ref, cim_ref, dsk_ref, gw_ref,
            o_ref,
            qt_s, k_s, vt_s, y_s, ure_s, uim_s, ot_s, m_s, l_s, *sbufs):
    i = pl.program_id(0)

    @pl.when(i == 0)
    def _prologue():
        x = x_ref[...]
        q = jnp.dot(x, wq_ref[...], preferred_element_type=jnp.float32) * (DH ** -0.5)
        qt_s[...] = _bf(q.T)
        k_s[...] = _bf(jnp.dot(x, wk_ref[...], preferred_element_type=jnp.float32))
        v = jnp.dot(x, wv_ref[...], preferred_element_type=jnp.float32)
        vt_s[...] = _bf(v.T)

        lr = lre_ref[...].astype(jnp.float32).reshape(1, -1)
        li = lim_ref[...].astype(jnp.float32).reshape(1, -1)
        dt = _bf(jnp.exp(ldt_ref[...].astype(jnp.float32).reshape(1, -1))).astype(jnp.float32)
        mag = jnp.exp(dt * lr)
        ang = dt * li
        lb_re = mag * jnp.cos(ang)
        lb_im = mag * jnp.sin(ang)
        nr = lb_re - 1.0
        ni = lb_im
        den = lr * lr + li * li
        cf_re = (nr * lr + ni * li) / den
        cf_im = (ni * lr - nr * li) / den

        xp = _bf(x.astype(jnp.float32).reshape(NSEG, SEGLEN, D).swapaxes(0, 1).reshape(S, D))

        u_re = jax.lax.dot_general(xp, bre_ref[...], _NT, preferred_element_type=jnp.float32)
        u_im = jax.lax.dot_general(xp, bim_ref[...], _NT, preferred_element_type=jnp.float32)
        ure_s[...] = cf_re * u_re - cf_im * u_im
        uim_s[...] = cf_re * u_im + cf_im * u_re

        lbr = jnp.broadcast_to(lb_re, (NSEG, P))
        lbi = jnp.broadcast_to(lb_im, (NSEG, P))

        def rows(j):
            return pl.ds(pl.multiple_of(j * NSEG, NSEG), NSEG)

        def local_step(j, c):
            hr, hi = c
            return (lbr * hr - lbi * hi + ure_s[rows(j), :],
                    lbr * hi + lbi * hr + uim_s[rows(j), :])

        z = jnp.zeros((NSEG, P), jnp.float32)
        er, ei = jax.lax.fori_loop(0, SEGLEN, local_step, (z, z), unroll=8)

        pr, pi_ = lb_re, lb_im
        for _ in range(8):
            pr, pi_ = pr * pr - pi_ * pi_, 2.0 * pr * pi_
        cr = jnp.zeros((1, P), jnp.float32)
        ci = jnp.zeros((1, P), jnp.float32)
        rr, ri = [cr], [ci]
        for sgi in range(1, NSEG):
            e_r = er[sgi - 1:sgi, :]
            e_i = ei[sgi - 1:sgi, :]
            cr, ci = pr * cr - pi_ * ci + e_r, pr * ci + pi_ * cr + e_i
            rr.append(cr)
            ri.append(ci)
        h0r = jnp.concatenate(rr, axis=0)
        h0i = jnp.concatenate(ri, axis=0)

        def true_step(j, c):
            hr, hi = c
            nhr = lbr * hr - lbi * hi + ure_s[rows(j), :]
            nhi = lbr * hi + lbi * hr + uim_s[rows(j), :]
            ure_s[rows(j), :] = nhr
            uim_s[rows(j), :] = nhi
            return (nhr, nhi)

        jax.lax.fori_loop(0, SEGLEN, true_step, (h0r, h0i), unroll=8)

        yy = (jax.lax.dot_general(_bf(ure_s[...]), cre_ref[...], _NT, preferred_element_type=jnp.float32)
              - jax.lax.dot_general(_bf(uim_s[...]), cim_ref[...], _NT, preferred_element_type=jnp.float32))
        yy = yy.reshape(SEGLEN, NSEG, D).swapaxes(0, 1).reshape(S, D)
        skip = _bf(x.astype(jnp.float32) * dsk_ref[...].astype(jnp.float32).reshape(1, -1)).astype(jnp.float32)
        y_s[...] = 2.0 * yy + skip

    q0 = pl.multiple_of(i * NQ, NQ)
    nck = S // CK
    nb = H // LA

    def stage(qb_qk, h_qk, dst, h_sm, src, m):
        if dst is not None:
            qtn = qt_s[pl.ds(pl.multiple_of(h_qk * DH, DH), DH),
                       pl.ds(pl.multiple_of(qb_qk * NQ, NQ), NQ)]
        if src is not None:
            acc = jnp.zeros((DH, NQ), jnp.float32)
        mrun = None
        for c in range(nck):
            if src is not None:
                p = jnp.exp(src[pl.ds(c * CK, CK), :] - m)
                l_s[pl.ds(8 * c, 8), :] = jnp.sum(p.reshape(CK // 8, 8, NQ), axis=0)
                acc = acc + jnp.dot(vt_s[:, pl.ds(c * CK, CK)], _bf(p),
                                    preferred_element_type=jnp.float32)
            if dst is not None:
                sn = jnp.dot(k_s[pl.ds(c * CK, CK), :], qtn, preferred_element_type=jnp.float32)
                dst[pl.ds(c * CK, CK), :] = sn
                cm = jnp.max(sn.reshape(CK // 8, 8, NQ), axis=0)
                mrun = cm if mrun is None else jnp.maximum(mrun, cm)
        if src is not None:
            ot_s[pl.ds(pl.multiple_of(h_sm * DH, DH), DH), :] = (
                acc / jnp.sum(l_s[...], axis=0, keepdims=True))
        if dst is not None:
            return jnp.max(mrun, axis=0, keepdims=True)
        return None

    bufs = sbufs

    @pl.when(i == 0)
    def _fill():
        for j in range(LA):
            m_s[pl.ds(j, 1), :] = stage(0, j, bufs[j], None, None, None)

    def block(b, par, ms):
        cur = bufs[par * LA:(par + 1) * LA]
        nxt = bufs[(1 - par) * LA:(2 - par) * LA]
        out = []
        for j in range(LA):
            t = b * LA + j + LA
            wrap = (t >= H).astype(jnp.int32)
            qb_n = jnp.minimum(i + wrap, S // NQ - 1)
            out.append(stage(qb_n, t - H * wrap, nxt[j], b * LA + j, cur[j], ms[j]))
        return tuple(out)

    ms = tuple(m_s[pl.ds(j, 1), :] for j in range(LA))
    ms = jax.lax.fori_loop(
        0, nb,
        lambda b, mm: jax.lax.cond(b % 2 == 0,
                                   lambda z: block(b, 0, z),
                                   lambda z: block(b, 1, z), mm),
        ms)
    for j in range(LA):
        m_s[pl.ds(j, 1), :] = ms[j]

    o_blk = _bf(ot_s[...].T)
    a = jnp.dot(o_blk, wo_ref[...], preferred_element_type=jnp.float32)
    xb = x_ref[pl.ds(q0, NQ), :].astype(jnp.float32)
    logit = jnp.sum(xb * gw_ref[...].astype(jnp.float32).reshape(1, -1), axis=-1, keepdims=True)
    g = jax.nn.sigmoid(logit)
    o_ref[...] = g * a + (1.0 - g) * y_s[pl.ds(q0, NQ), :]


@jax.jit
def pallas_gated_mix__grouped_kv_mqa__ssm_conv_s5__prompt_kernel(
    A_x, A_wq, A_wk, A_wv, A_wo, B_x, B_Lambda_re, B_Lambda_im, B_B_re, B_B_im,
    B_C_re, B_C_im, B_log_dt, B_Dskip, gate_w,
):
    x = A_x.reshape(S, D)

    def full(shape):
        return pl.BlockSpec(shape, lambda i: (0,) * len(shape))

    out = pl.pallas_call(
        _kernel,
        grid=(S // NQ,),
        in_specs=[full((S, D)), full((D, H * DH)), full((D, DH)), full((D, DH)),
                  full((H * DH, D)), full((P,)), full((P,)), full((P,)),
                  full((P, D)), full((P, D)), full((D, P)), full((D, P)),
                  full((D,)), full((D,))],
        out_specs=pl.BlockSpec((NQ, D), lambda i: (i, 0)),
        out_shape=jax.ShapeDtypeStruct((S, D), jnp.float32),
        scratch_shapes=[
            pltpu.VMEM((H * DH, S), jnp.bfloat16),
            pltpu.VMEM((S, DH), jnp.bfloat16),
            pltpu.VMEM((DH, S), jnp.bfloat16),
            pltpu.VMEM((S, D), jnp.float32),
            pltpu.VMEM((S, P), jnp.float32),
            pltpu.VMEM((S, P), jnp.float32),
            pltpu.VMEM((H * DH, NQ), jnp.float32),
            pltpu.VMEM((8, NQ), jnp.float32),
            pltpu.VMEM((8 * (S // CK), NQ), jnp.float32),
        ] + [pltpu.VMEM((S, NQ), jnp.float32) for _ in range(2 * LA)],

        compiler_params=pltpu.CompilerParams(
            dimension_semantics=("arbitrary",),
            vmem_limit_bytes=112 * 1024 * 1024),
    )(x, A_wq, A_wk, A_wv, A_wo, B_Lambda_re, B_Lambda_im, B_log_dt,
      B_B_re, B_B_im, B_C_re, B_C_im, B_Dskip, gate_w)
    return out.reshape(1, S, D)
```

```python
import jax
import jax.numpy as jnp
import jax.experimental.pallas as pl
import jax.experimental.pallas.tpu as pltpu

S = 2048
D = 512
H = 32
DH = 16
P = 512
NQ = 512
CK = 128
LA = 2
NSEG = 8
SEGLEN = S // NSEG

_NT = (((1,), (1,)), ((), ()))


def _bf(v):
    return v.astype(jnp.bfloat16)


def _kernel(x_ref, wq_ref, wk_ref, wv_ref, wo_ref, lre_ref, lim_ref, ldt_ref,
            bre_ref, bim_ref, cre_ref, cim_ref, dsk_ref, gw_ref,
            o_ref,
            qt_s, k_s, vt_s, y_s, ure_s, uim_s, ot_s, m_s, l_s, wbig_s, wsem, *sbufs):
    i = pl.program_id(0)

    @pl.when(i == 0)
    def _prologue():
        cps = [pltpu.make_async_copy(src, wbig_s.at[n], wsem.at[n])
               for n, src in enumerate((bre_ref, bim_ref, cre_ref, cim_ref, wo_ref))]
        for cp in cps:
            cp.start()
        x = x_ref[...]
        q = jnp.dot(x, wq_ref[...], preferred_element_type=jnp.float32) * (DH ** -0.5)
        qt_s[...] = _bf(q.T)
        k_s[...] = _bf(jnp.dot(x, wk_ref[...], preferred_element_type=jnp.float32))
        v = jnp.dot(x, wv_ref[...], preferred_element_type=jnp.float32)
        vt_s[...] = _bf(v.T)

        lr = lre_ref[...].astype(jnp.float32).reshape(1, -1)
        li = lim_ref[...].astype(jnp.float32).reshape(1, -1)
        dt = _bf(jnp.exp(ldt_ref[...].astype(jnp.float32).reshape(1, -1))).astype(jnp.float32)
        mag = jnp.exp(dt * lr)
        ang = dt * li
        lb_re = mag * jnp.cos(ang)
        lb_im = mag * jnp.sin(ang)
        nr = lb_re - 1.0
        ni = lb_im
        den = lr * lr + li * li
        cf_re = (nr * lr + ni * li) / den
        cf_im = (ni * lr - nr * li) / den

        xp = _bf(x.astype(jnp.float32).reshape(NSEG, SEGLEN, D).swapaxes(0, 1).reshape(S, D))

        cps[0].wait()
        u_re = jax.lax.dot_general(xp, wbig_s[0], _NT, preferred_element_type=jnp.float32)
        cps[1].wait()
        u_im = jax.lax.dot_general(xp, wbig_s[1], _NT, preferred_element_type=jnp.float32)
        ure_s[...] = cf_re * u_re - cf_im * u_im
        uim_s[...] = cf_re * u_im + cf_im * u_re

        lbr = jnp.broadcast_to(lb_re, (NSEG, P))
        lbi = jnp.broadcast_to(lb_im, (NSEG, P))

        def rows(j):
            return pl.ds(pl.multiple_of(j * NSEG, NSEG), NSEG)

        def local_step(j, c):
            hr, hi = c
            return (lbr * hr - lbi * hi + ure_s[rows(j), :],
                    lbr * hi + lbi * hr + uim_s[rows(j), :])

        z = jnp.zeros((NSEG, P), jnp.float32)
        er, ei = jax.lax.fori_loop(0, SEGLEN, local_step, (z, z), unroll=8)

        pr, pi_ = lb_re, lb_im
        for _ in range(8):
            pr, pi_ = pr * pr - pi_ * pi_, 2.0 * pr * pi_
        cr = jnp.zeros((1, P), jnp.float32)
        ci = jnp.zeros((1, P), jnp.float32)
        rr, ri = [cr], [ci]
        for sgi in range(1, NSEG):
            e_r = er[sgi - 1:sgi, :]
            e_i = ei[sgi - 1:sgi, :]
            cr, ci = pr * cr - pi_ * ci + e_r, pr * ci + pi_ * cr + e_i
            rr.append(cr)
            ri.append(ci)
        h0r = jnp.concatenate(rr, axis=0)
        h0i = jnp.concatenate(ri, axis=0)

        def true_step(j, c):
            hr, hi = c
            nhr = lbr * hr - lbi * hi + ure_s[rows(j), :]
            nhi = lbr * hi + lbi * hr + uim_s[rows(j), :]
            ure_s[rows(j), :] = nhr
            uim_s[rows(j), :] = nhi
            return (nhr, nhi)

        jax.lax.fori_loop(0, SEGLEN, true_step, (h0r, h0i), unroll=8)

        cps[2].wait()
        cps[3].wait()
        cps[4].wait()
        yy = (jax.lax.dot_general(_bf(ure_s[...]), wbig_s[2], _NT, preferred_element_type=jnp.float32)
              - jax.lax.dot_general(_bf(uim_s[...]), wbig_s[3], _NT, preferred_element_type=jnp.float32))
        yy = yy.reshape(SEGLEN, NSEG, D).swapaxes(0, 1).reshape(S, D)
        skip = _bf(x.astype(jnp.float32) * dsk_ref[...].astype(jnp.float32).reshape(1, -1)).astype(jnp.float32)
        y_s[...] = 2.0 * yy + skip

    q0 = pl.multiple_of(i * NQ, NQ)
    nck = S // CK
    nb = H // LA

    def stage(qb_qk, h_qk, dst, h_sm, src, m):
        if dst is not None:
            qtn = qt_s[pl.ds(pl.multiple_of(h_qk * DH, DH), DH),
                       pl.ds(pl.multiple_of(qb_qk * NQ, NQ), NQ)]
        if src is not None:
            acc = jnp.zeros((DH, NQ), jnp.float32)
        mrun = None
        for c in range(nck):
            if src is not None:
                p = jnp.exp(src[pl.ds(c * CK, CK), :] - m)
                l_s[pl.ds(8 * c, 8), :] = jnp.sum(p.reshape(CK // 8, 8, NQ), axis=0)
                acc = acc + jnp.dot(vt_s[:, pl.ds(c * CK, CK)], _bf(p),
                                    preferred_element_type=jnp.float32)
            if dst is not None:
                sn = jnp.dot(k_s[pl.ds(c * CK, CK), :], qtn, preferred_element_type=jnp.float32)
                dst[pl.ds(c * CK, CK), :] = sn
                cm = jnp.max(sn.reshape(CK // 8, 8, NQ), axis=0)
                mrun = cm if mrun is None else jnp.maximum(mrun, cm)
        if src is not None:
            ot_s[pl.ds(pl.multiple_of(h_sm * DH, DH), DH), :] = (
                acc / jnp.sum(l_s[...], axis=0, keepdims=True))
        if dst is not None:
            return jnp.max(mrun, axis=0, keepdims=True)
        return None

    bufs = sbufs

    @pl.when(i == 0)
    def _fill():
        for j in range(LA):
            m_s[pl.ds(j, 1), :] = stage(0, j, bufs[j], None, None, None)

    def block(b, par, ms):
        cur = bufs[par * LA:(par + 1) * LA]
        nxt = bufs[(1 - par) * LA:(2 - par) * LA]
        out = []
        for j in range(LA):
            t = b * LA + j + LA
            wrap = (t >= H).astype(jnp.int32)
            qb_n = jnp.minimum(i + wrap, S // NQ - 1)
            out.append(stage(qb_n, t - H * wrap, nxt[j], b * LA + j, cur[j], ms[j]))
        return tuple(out)

    ms = tuple(m_s[pl.ds(j, 1), :] for j in range(LA))
    ms = jax.lax.fori_loop(
        0, nb,
        lambda b, mm: jax.lax.cond(b % 2 == 0,
                                   lambda z: block(b, 0, z),
                                   lambda z: block(b, 1, z), mm),
        ms)
    for j in range(LA):
        m_s[pl.ds(j, 1), :] = ms[j]

    o_blk = _bf(ot_s[...].T)
    a = jnp.dot(o_blk, wbig_s[4], preferred_element_type=jnp.float32)
    xb = x_ref[pl.ds(q0, NQ), :].astype(jnp.float32)
    logit = jnp.sum(xb * gw_ref[...].astype(jnp.float32).reshape(1, -1), axis=-1, keepdims=True)
    g = jax.nn.sigmoid(logit)
    o_ref[...] = g * a + (1.0 - g) * y_s[pl.ds(q0, NQ), :]


@jax.jit
def pallas_gated_mix__grouped_kv_mqa__ssm_conv_s5__prompt_kernel(
    A_x, A_wq, A_wk, A_wv, A_wo, B_x, B_Lambda_re, B_Lambda_im, B_B_re, B_B_im,
    B_C_re, B_C_im, B_log_dt, B_Dskip, gate_w,
):
    x = A_x.reshape(S, D)

    def full(shape):
        return pl.BlockSpec(shape, lambda i: (0,) * len(shape))

    out = pl.pallas_call(
        _kernel,
        grid=(S // NQ,),
        in_specs=[full((S, D)), full((D, H * DH)), full((D, DH)), full((D, DH)),
                  pl.BlockSpec(memory_space=pl.ANY), full((P,)), full((P,)), full((P,)),
                  pl.BlockSpec(memory_space=pl.ANY), pl.BlockSpec(memory_space=pl.ANY),
                  pl.BlockSpec(memory_space=pl.ANY), pl.BlockSpec(memory_space=pl.ANY),
                  full((D,)), full((D,))],
        out_specs=pl.BlockSpec((NQ, D), lambda i: (i, 0)),
        out_shape=jax.ShapeDtypeStruct((S, D), jnp.float32),
        scratch_shapes=[
            pltpu.VMEM((H * DH, S), jnp.bfloat16),
            pltpu.VMEM((S, DH), jnp.bfloat16),
            pltpu.VMEM((DH, S), jnp.bfloat16),
            pltpu.VMEM((S, D), jnp.float32),
            pltpu.VMEM((S, P), jnp.float32),
            pltpu.VMEM((S, P), jnp.float32),
            pltpu.VMEM((H * DH, NQ), jnp.float32),
            pltpu.VMEM((8, NQ), jnp.float32),
            pltpu.VMEM((8 * (S // CK), NQ), jnp.float32),
            pltpu.VMEM((5, D, D), jnp.bfloat16),
            pltpu.SemaphoreType.DMA((5,)),
        ] + [pltpu.VMEM((S, NQ), jnp.float32) for _ in range(2 * LA)],

        compiler_params=pltpu.CompilerParams(
            dimension_semantics=("arbitrary",),
            vmem_limit_bytes=112 * 1024 * 1024),
    )(x, A_wq, A_wk, A_wv, A_wo, B_Lambda_re, B_Lambda_im, B_log_dt,
      B_B_re, B_B_im, B_C_re, B_C_im, B_Dskip, gate_w)
    return out.reshape(1, S, D)
```
